```python
import os as _os
_os.environ.setdefault("JAX_PLATFORMS", "cpu")
import jax
import jax.numpy as jnp

def _softmax(x, axis=-1):
    return jax.nn.softmax(x, axis=axis)
def _gelu(x):
    return jax.nn.gelu(x, approximate=True)
def _silu(x):
    return jax.nn.silu(x)
def _sigmoid(x):
    return jax.nn.sigmoid(x)
def _layernorm(x, axis=-1, eps=1e-5):
    m = jnp.mean(x, axis=axis, keepdims=True)
    v = jnp.var(x, axis=axis, keepdims=True)
    return (x - m) / jnp.sqrt(v + eps)
def _scatter_add(tgt, idx, src, axis=0):
    return tgt.at[idx].add(src)
def _segment_sum(src, seg, n):
    return jax.ops.segment_sum(src, seg, n)
class _Rng:
    def __init__(self, key):
        self._k = key
    def _next(self):
        self._k, sub = jax.random.split(self._k)
        return sub
    def normal(self, shape):
        return jax.random.normal(self._next(), shape, dtype=jnp.bfloat16)
    def randint(self, lo, hi, shape):
        return jax.random.randint(self._next(), shape, lo, hi, dtype=jnp.int32)
    def uniform(self, shape, lo=0.0, hi=1.0):
        return jax.random.uniform(self._next(), shape, jnp.bfloat16, lo, hi)
    def permutation(self, n):
        return jax.random.permutation(self._next(), n)


kernel_name = 'parallel_sum__softmax_full_mha__swiglu_ffn__prompt'

def setup_inputs():
    _rng = _Rng(jax.random.key(int.from_bytes(__import__("os").urandom(4), "little")))
    _w = (lambda a: (lambda t: t.astype(jnp.bfloat16) if jnp.issubdtype(t.dtype, jnp.floating) else t)(jnp.asarray(a)))
    def _A_setup():
        B, S, D = 1, 2048, 640
        return {
            "x": _w((lambda *s: _rng.normal(s) * 0.05)(B, S, D)),
            "wqkv": _w((lambda *s: _rng.normal(s) * 0.1)(D, 3 * D)),
            "wo": _w((lambda *s: _rng.normal(s) * 0.05)(D, D)),
        }
    _A_in = _A_setup()

    def _B_setup():
        B, S, D, F = 1, 2048, 640, 1536
        return {
            "x": _w((lambda *s: _rng.normal(s) * 0.05)(B, S, D)),
            "w_gate": _w((lambda *s: _rng.normal(s) * 0.05)(D, F)),
            "w_up": _w((lambda *s: _rng.normal(s) * 0.05)(D, F)),
            "w_down": _w((lambda *s: _rng.normal(s) * 0.05)(F, D)),
        }
    _B_in = _B_setup()

    return {
        "A_x": _A_in["x"],
        "A_wqkv": _A_in["wqkv"],
        "A_wo": _A_in["wo"],
        "B_x": _B_in["x"],
        "B_w_gate": _B_in["w_gate"],
        "B_w_up": _B_in["w_up"],
        "B_w_down": _B_in["w_down"],
    }

def reference(A_x, A_wqkv, A_wo, B_x, B_w_gate, B_w_up, B_w_down):
    def _A_ref(x, wqkv, wo):
        B, S, D = x.shape
        H = 32; Dh = D // H
        qkv = (lambda x, *d: x.transpose(*d))((x @ wqkv).reshape(B, S, 3, H, Dh), 2, 0, 3, 1, 4)
        q, k, v = qkv[0], qkv[1], qkv[2]
        scale = Dh ** -0.5
        scores = jnp.einsum("bhqd,bhkd->bhqk", q, k) * scale
        p = _softmax(scores, axis=-1)
        o = jnp.einsum("bhqk,bhkd->bhqd", p, v)
        return (lambda x, *d: x.transpose(*d))(o, 0, 2, 1, 3).reshape(B, S, D) @ wo

    def _B_ref(x, w_gate, w_up, w_down):
        g = _silu(x @ w_gate)
        u = x @ w_up
        return (g * u) @ w_down

    x = A_x
    xn = _layernorm(x, axis=-1)
    return x + _A_ref(xn, A_wqkv, A_wo) + _B_ref(xn, B_w_gate, B_w_up, B_w_down)
```

```python
import math

import jax
import jax.numpy as jnp
from jax import lax
import jax.experimental.pallas as pl
import jax.experimental.pallas.tpu as pltpu

S, D, H, DH, F = 2048, 640, 32, 20, 1536
NBLK = 6
VP = 32
OP = 24
TQ = 512
CK = 128
FUSE_FFN = True
NQ = S // TQ
NSTEP = H * NQ
GU_ROWS = TQ // 2
N_GU = (S // GU_ROWS) * (F // 128)
DN_ROWS = S // (NSTEP - N_GU)
F32, BF16 = jnp.float32, jnp.bfloat16


def _dot(a, b):
    return jnp.dot(a, b, preferred_element_type=F32)


def _kernel(x_ref, wqkv_ref, wo_hbm, wg_hbm, wu_hbm, wd_hbm, out_ref,
            wo_ref, wg_ref, wu_ref, wd_ref, sems,
            xn_ref, k_ref, qt_ref, vt_ref, ot_ref, wop_ref, h_ref, ffn_ref,
            s0, s1, p0, p1):
    copies = [pltpu.make_async_copy(src, dst, sems.at[i]) for i, (src, dst) in enumerate(
        ((wg_hbm, wg_ref), (wu_hbm, wu_ref), (wd_hbm, wd_ref), (wo_hbm, wo_ref)))]
    for c in copies:
        c.start()

    def ln(i, _):
        r = pl.ds(pl.multiple_of(i * 256, 256), 256)
        x = x_ref[r, :].astype(F32)
        xc = x - jnp.mean(x, axis=-1, keepdims=True)
        v = jnp.mean(xc * xc, axis=-1, keepdims=True)
        xn_ref[r, :] = (xc * lax.rsqrt(v + 1e-5)).astype(BF16)
        return _
    lax.fori_loop(0, S // 256, ln, 0)

    tn = (((0,), (1,)), ((), ()))
    qscale = DH ** -0.5 * math.log2(math.e)
    wq = wqkv_ref[:, 0:D]
    wk = wqkv_ref[:, D:2 * D]
    for b in range(NBLK):
        off = min(120 * b, D - 128)
        k_ref[:, b * 128:(b + 1) * 128] = _dot(xn_ref[...], wk[:, off:off + 128]).astype(BF16)
        qt = lax.dot_general(wq[:, off:off + 128], xn_ref[...], tn, preferred_element_type=F32)
        qt_ref[b * 128:(b + 1) * 128, :] = (qt * qscale).astype(BF16)
    for b in range(D // 128):
        ot_ref[b * 128:(b + 1) * 128, :] = lax.dot_general(
            wqkv_ref[:, 2 * D + b * 128:2 * D + (b + 1) * 128], xn_ref[...], tn,
            preferred_element_type=F32)
    row = lax.broadcasted_iota(jnp.int32, (VP - DH, S), 0)
    tail = jnp.where(row == 0, 1.0, 0.0).astype(F32)
    for h in range(H):
        v = jnp.concatenate([ot_ref[h * DH:(h + 1) * DH, :], tail], axis=0)
        vt_ref[h * VP:(h + 1) * VP, :] = v.astype(BF16)

    for c in copies[:3]:
        c.wait()

    def gate_up(u):
        r = pl.ds(pl.multiple_of((u // (F // 128)) * GU_ROWS, GU_ROWS), GU_ROWS)
        c = pl.ds(pl.multiple_of((u % (F // 128)) * 128, 128), 128)
        xr = xn_ref[r, :]
        g = _dot(xr, wg_ref[:, c])
        up = _dot(xr, wu_ref[:, c])
        h_ref[r, c] = (g * jax.nn.sigmoid(g) * up).astype(BF16)

    def down(u):
        r = pl.ds(pl.multiple_of(u * DN_ROWS, DN_ROWS), DN_ROWS)
        ffn_ref[r, :] = _dot(h_ref[r, :], wd_ref[...])

    def getq(i):
        h = i // NQ
        q0 = pl.multiple_of((i % NQ) * TQ, TQ)
        blk = jnp.minimum(h // 6, NBLK - 1)
        lo = h * DH - jnp.minimum(blk * 120, D - 128)
        lane0 = pl.multiple_of(blk * 128, 128)
        qb = qt_ref[pl.ds(lane0, 128), pl.ds(q0, TQ)]
        r = lax.broadcasted_iota(jnp.int32, qb.shape, 0)
        return jnp.where((r >= lo) & (r < lo + DH), qb, jnp.zeros_like(qb)), lane0

    def scores(i, sref):
        qh, lane0 = getq(i)
        s = _dot(k_ref[:, pl.ds(lane0, 128)], qh)
        sref[...] = s
        return jnp.max(s, axis=0, keepdims=True)

    def step(i, sa, sb, pb, pc, mb, extra):
        qh, lane0 = getq(jnp.minimum(i + 2, NSTEP - 1))
        hc = i // NQ
        vrow = pl.ds(pl.multiple_of(hc * VP, VP), VP)
        ma = acc = None
        for c in range(S // CK):
            ck = pl.ds(c * CK, CK)
            s = _dot(k_ref[ck, pl.ds(lane0, 128)], qh)
            sa[ck, :] = s
            mm = jnp.max(s.reshape(CK // 8, 8, TQ), axis=0)
            ma = mm if ma is None else jnp.maximum(ma, mm)
            pb[ck, :] = jnp.exp2(sb[ck, :] - mb).astype(BF16)
            o = _dot(vt_ref[vrow, ck], pc[ck, :])
            acc = o if acc is None else acc + o
        ot_ref[pl.ds(pl.multiple_of(hc * OP, 8), OP), pl.ds(pl.multiple_of((i % NQ) * TQ, TQ), TQ)] = (
            acc[0:OP] / acc[DH:DH + 1])
        extra(i)
        return jnp.max(ma, axis=0, keepdims=True)

    def run(lo, hi, m, extra):
        def body(j, m):
            m = step(2 * j, s0, s1, p1, p0, m, extra)
            return step(2 * j + 1, s1, s0, p0, p1, m, extra)
        return lax.fori_loop(lo // 2, hi // 2, body, m)

    m0 = scores(0, s0)
    p0[...] = jnp.exp2(s0[...] - m0).astype(BF16)
    m = scores(1, s1)
    if FUSE_FFN:
        m = run(0, N_GU, m, gate_up)
        run(N_GU, NSTEP, m, lambda i: down(i - N_GU))
    else:
        run(0, NSTEP, m, lambda i: None)
        lax.fori_loop(0, N_GU, lambda u, c: (gate_up(u), c)[1], 0)
        lax.fori_loop(0, NSTEP - N_GU, lambda u, c: (down(u), c)[1], 0)

    copies[3].wait()
    wop_ref[...] = jnp.zeros(wop_ref.shape, F32)
    wo = wo_ref[...].astype(F32)
    for h in range(H):
        wop_ref[h * OP:h * OP + DH, :] = wo[h * DH:(h + 1) * DH, :]
    wop = wop_ref[...].astype(BF16)

    def fin(i, _):
        r0 = pl.multiple_of(i * 512, 512)
        r = pl.ds(r0, 512)
        a = lax.dot_general(ot_ref[:, r].astype(BF16), wop, (((0,), (0,)), ((), ())),
                            preferred_element_type=F32)
        out_ref[r, :] = (x_ref[r, :].astype(F32) + a + ffn_ref[r, :]).astype(BF16)
        return _
    lax.fori_loop(0, S // 512, fin, 0)


@jax.jit
def pallas_parallel_sum__softmax_full_mha__swiglu_ffn__prompt_kernel(
    A_x, A_wqkv, A_wo, B_x, B_w_gate, B_w_up, B_w_down,
):
    del B_x
    vm = pl.BlockSpec(memory_space=pltpu.VMEM)
    hbm = pl.BlockSpec(memory_space=pl.ANY)
    V = pltpu.VMEM
    out = pl.pallas_call(
        _kernel,
        out_shape=jax.ShapeDtypeStruct((S, D), BF16),
        in_specs=[vm, vm, hbm, hbm, hbm, hbm],
        out_specs=vm,
        scratch_shapes=[
            V((D, D), BF16), V((D, F), BF16), V((D, F), BF16), V((F, D), BF16),
            pltpu.SemaphoreType.DMA((4,)),
            V((S, D), BF16), V((S, NBLK * 128), BF16), V((NBLK * 128, S), BF16),
            V((H * VP, S), BF16), V((H * OP, S), F32), V((H * OP, D), F32),
            V((S, F), BF16), V((S, D), F32),
            V((S, TQ), F32), V((S, TQ), F32), V((S, TQ), BF16), V((S, TQ), BF16),
        ],
        compiler_params=pltpu.CompilerParams(vmem_limit_bytes=110 * 2**20),
    )(A_x.reshape(S, D), A_wqkv, A_wo, B_w_gate, B_w_up, B_w_down)
    return out.reshape(1, S, D)
```

```python
import math

import jax
import jax.numpy as jnp
from jax import lax
import jax.experimental.pallas as pl
import jax.experimental.pallas.tpu as pltpu

S, D, H, DH, F = 2048, 640, 32, 20, 1536
NBLK = 6
VP = 32
OP = 24
TQ = 512
CK = 128
FUSE_FFN = True
NQ = S // TQ
NSTEP = H * NQ
GU_ROWS = TQ // 2
N_GU = (S // GU_ROWS) * (F // 128)
DN_ROWS = S // (NSTEP - N_GU)
F32, BF16 = jnp.float32, jnp.bfloat16


def _dot(a, b):
    return jnp.dot(a, b, preferred_element_type=F32)


def _kernel(x_ref, wqkv_hbm, wo_hbm, wg_hbm, wu_hbm, wd_hbm, out_hbm,
            wqkv_ref, out_ref, q0_ref, q1_ref, osems, wo_ref, wg_ref, wu_ref, wd_ref, sems,
            xn_ref, k_ref, qt_ref, vt_ref, ot_ref, wop_ref, h_ref, ffn_ref,
            s0, s1, p0, p1):
    copies = [pltpu.make_async_copy(src, dst, sems.at[i]) for i, (src, dst) in enumerate(
        ((wg_hbm, wg_ref), (wu_hbm, wu_ref), (wd_hbm, wd_ref), (wo_hbm, wo_ref),
         (wqkv_hbm, wqkv_ref)))]
    for c in copies[::-1]:
        c.start()

    def ln(i, _):
        r = pl.ds(pl.multiple_of(i * 256, 256), 256)
        x = x_ref[r, :].astype(F32)
        xc = x - jnp.mean(x, axis=-1, keepdims=True)
        v = jnp.mean(xc * xc, axis=-1, keepdims=True)
        xn_ref[r, :] = (xc * lax.rsqrt(v + 1e-5)).astype(BF16)
        return _
    lax.fori_loop(0, S // 256, ln, 0)

    tn = (((0,), (1,)), ((), ()))
    qscale = DH ** -0.5 * math.log2(math.e)
    copies[4].wait()
    wq = wqkv_ref[:, 0:D]
    wk = wqkv_ref[:, D:2 * D]
    for b in range(NBLK):
        off = min(120 * b, D - 128)
        k_ref[:, b * 128:(b + 1) * 128] = _dot(xn_ref[...], wk[:, off:off + 128]).astype(BF16)
        qt = lax.dot_general(wq[:, off:off + 128], xn_ref[...], tn, preferred_element_type=F32)
        qt_ref[b * 128:(b + 1) * 128, :] = (qt * qscale).astype(BF16)
    for b in range(D // 128):
        ot_ref[b * 128:(b + 1) * 128, :] = lax.dot_general(
            wqkv_ref[:, 2 * D + b * 128:2 * D + (b + 1) * 128], xn_ref[...], tn,
            preferred_element_type=F32)
    row = lax.broadcasted_iota(jnp.int32, (VP - DH, S), 0)
    tail = jnp.where(row == 0, 1.0, 0.0).astype(F32)
    for h in range(H):
        v = jnp.concatenate([ot_ref[h * DH:(h + 1) * DH, :], tail], axis=0)
        vt_ref[h * VP:(h + 1) * VP, :] = v.astype(BF16)

    copies[3].wait()
    wop_ref[...] = jnp.zeros(wop_ref.shape, F32)
    wo = wo_ref[...].astype(F32)
    for h in range(H):
        wop_ref[h * OP:h * OP + DH, :] = wo[h * DH:(h + 1) * DH, :]
    for c in copies[:3]:
        c.wait()

    def gate_up(u):
        r = pl.ds(pl.multiple_of((u // (F // 128)) * GU_ROWS, GU_ROWS), GU_ROWS)
        c = pl.ds(pl.multiple_of((u % (F // 128)) * 128, 128), 128)
        xr = xn_ref[r, :]
        g = _dot(xr, wg_ref[:, c])
        up = _dot(xr, wu_ref[:, c])
        h_ref[r, c] = (g * jax.nn.sigmoid(g) * up).astype(BF16)

    def down(u):
        r = pl.ds(pl.multiple_of(u * DN_ROWS, DN_ROWS), DN_ROWS)
        ffn_ref[r, :] = _dot(h_ref[r, :], wd_ref[...])

    def getq(i):
        h = i // NQ
        q0 = pl.multiple_of((i % NQ) * TQ, TQ)
        blk = jnp.minimum(h // 6, NBLK - 1)
        lo = h * DH - jnp.minimum(blk * 120, D - 128)
        lane0 = pl.multiple_of(blk * 128, 128)
        qb = qt_ref[pl.ds(lane0, 128), pl.ds(q0, TQ)]
        r = lax.broadcasted_iota(jnp.int32, qb.shape, 0)
        return jnp.where((r >= lo) & (r < lo + DH), qb, jnp.zeros_like(qb)), lane0

    def scores(i, sref):
        qh, lane0 = getq(i)
        s = _dot(k_ref[:, pl.ds(lane0, 128)], qh)
        sref[...] = s
        return jnp.max(s, axis=0, keepdims=True)

    def step(i, sa, sb, pb, pc, qc, qn, mb, extra):
        h2 = jnp.minimum(i + 2, NSTEP - 1) // NQ
        lane0 = pl.multiple_of(jnp.minimum(h2 // 6, NBLK - 1) * 128, 128)
        qh = qc[...]
        qn[...] = getq(jnp.minimum(i + 3, NSTEP - 1))[0]
        hc = i // NQ
        vrow = pl.ds(pl.multiple_of(hc * VP, VP), VP)
        ma = acc = None
        for c in range(S // CK):
            ck = pl.ds(c * CK, CK)
            s = _dot(k_ref[ck, pl.ds(lane0, 128)], qh)
            sa[ck, :] = s
            mm = jnp.max(s.reshape(CK // 8, 8, TQ), axis=0)
            ma = mm if ma is None else jnp.maximum(ma, mm)
            pb[ck, :] = jnp.exp2(sb[ck, :] - mb).astype(BF16)
            o = _dot(vt_ref[vrow, ck], pc[ck, :])
            acc = o if acc is None else acc + o
        ot_ref[pl.ds(pl.multiple_of(hc * OP, 8), OP), pl.ds(pl.multiple_of((i % NQ) * TQ, TQ), TQ)] = (
            acc[0:OP] / acc[DH:DH + 1])
        extra(i)
        return jnp.max(ma, axis=0, keepdims=True)

    def run(lo, hi, m, extra):
        def body(i, m):
            return lax.cond(i % 2 == 0,
                            lambda: step(i, s0, s1, p1, p0, q0_ref, q1_ref, m, extra),
                            lambda: step(i, s1, s0, p0, p1, q1_ref, q0_ref, m, extra))
        return lax.fori_loop(lo, hi, body, m)

    m0 = scores(0, s0)
    p0[...] = jnp.exp2(s0[...] - m0).astype(BF16)
    m = scores(1, s1)
    q0_ref[...] = getq(2)[0]
    if FUSE_FFN:
        m = run(0, N_GU, m, gate_up)
        run(N_GU, NSTEP, m, lambda i: down(i - N_GU))
    else:
        run(0, NSTEP, m, lambda i: None)
        lax.fori_loop(0, N_GU, lambda u, c: (gate_up(u), c)[1], 0)
        lax.fori_loop(0, NSTEP - N_GU, lambda u, c: (down(u), c)[1], 0)

    wop = wop_ref[...].astype(BF16)

    def fin(i):
        r0 = i * 512
        r = pl.ds(r0, 512)
        a = lax.dot_general(ot_ref[:, r].astype(BF16), wop, (((0,), (0,)), ((), ())),
                            preferred_element_type=F32)
        out_ref[r, :] = (x_ref[r, :].astype(F32) + a + ffn_ref[r, :]).astype(BF16)
    outs = []
    for i in range(S // 512):
        fin(i)
        r = pl.ds(i * 512, 512)
        outs.append(pltpu.make_async_copy(out_ref.at[r], out_hbm.at[r], osems.at[i]))
        outs[-1].start()
    for c in outs:
        c.wait()


@jax.jit
def pallas_parallel_sum__softmax_full_mha__swiglu_ffn__prompt_kernel(
    A_x, A_wqkv, A_wo, B_x, B_w_gate, B_w_up, B_w_down,
):
    del B_x
    vm = pl.BlockSpec(memory_space=pltpu.VMEM)
    hbm = pl.BlockSpec(memory_space=pl.ANY)
    V = pltpu.VMEM
    out = pl.pallas_call(
        _kernel,
        out_shape=jax.ShapeDtypeStruct((S, D), BF16),
        in_specs=[vm, hbm, hbm, hbm, hbm, hbm],
        out_specs=hbm,
        scratch_shapes=[
            V((D, 3 * D), BF16), V((S, D), BF16), V((128, TQ), BF16), V((128, TQ), BF16),
            pltpu.SemaphoreType.DMA((S // 512,)),
            V((D, D), BF16), V((D, F), BF16), V((D, F), BF16), V((F, D), BF16),
            pltpu.SemaphoreType.DMA((5,)),
            V((S, D), BF16), V((S, NBLK * 128), BF16), V((NBLK * 128, S), BF16),
            V((H * VP, S), BF16), V((H * OP, S), F32), V((H * OP, D), F32),
            V((S, F), BF16), V((S, D), F32),
            V((S, TQ), F32), V((S, TQ), F32), V((S, TQ), BF16), V((S, TQ), BF16),
        ],
        compiler_params=pltpu.CompilerParams(vmem_limit_bytes=110 * 2**20),
    )(A_x.reshape(S, D), A_wqkv, A_wo, B_w_gate, B_w_up, B_w_down)
    return out.reshape(1, S, D)
```
